```python
import os as _os
_os.environ.setdefault("JAX_PLATFORMS", "cpu")
import jax
import jax.numpy as jnp

def _softmax(x, axis=-1):
    return jax.nn.softmax(x, axis=axis)
def _gelu(x):
    return jax.nn.gelu(x, approximate=True)
def _silu(x):
    return jax.nn.silu(x)
def _sigmoid(x):
    return jax.nn.sigmoid(x)
def _layernorm(x, axis=-1, eps=1e-5):
    m = jnp.mean(x, axis=axis, keepdims=True)
    v = jnp.var(x, axis=axis, keepdims=True)
    return (x - m) / jnp.sqrt(v + eps)
def _scatter_add(tgt, idx, src, axis=0):
    return tgt.at[idx].add(src)
def _segment_sum(src, seg, n):
    return jax.ops.segment_sum(src, seg, n)
class _Rng:
    def __init__(self, key):
        self._k = key
    def _next(self):
        self._k, sub = jax.random.split(self._k)
        return sub
    def normal(self, shape):
        return jax.random.normal(self._next(), shape, dtype=jnp.bfloat16)
    def randint(self, lo, hi, shape):
        return jax.random.randint(self._next(), shape, lo, hi, dtype=jnp.int32)
    def uniform(self, shape, lo=0.0, hi=1.0):
        return jax.random.uniform(self._next(), shape, jnp.bfloat16, lo, hi)
    def permutation(self, n):
        return jax.random.permutation(self._next(), n)


kernel_name = 'sequential_preLN__softmax_full_mha__swiglu_ffn__prompt'

def setup_inputs():
    _rng = _Rng(jax.random.key(int.from_bytes(__import__("os").urandom(4), "little")))
    _w = (lambda a: (lambda t: t.astype(jnp.bfloat16) if jnp.issubdtype(t.dtype, jnp.floating) else t)(jnp.asarray(a)))
    def _A_setup():
        B, S, D = 1, 2048, 512
        return {
            "x": _w((lambda *s: _rng.normal(s) * 0.05)(B, S, D)),
            "wqkv": _w((lambda *s: _rng.normal(s) * 0.05)(D, 3 * D)),
            "wo": _w((lambda *s: _rng.normal(s) * 0.05)(D, D)),
        }
    _A_in = _A_setup()

    def _B_setup():
        B, S, D, F = 1, 2048, 512, 1792
        return {
            "x": _w((lambda *s: _rng.normal(s) * 0.05)(B, S, D)),
            "w_gate": _w((lambda *s: _rng.normal(s) * 0.05)(D, F)),
            "w_up": _w((lambda *s: _rng.normal(s) * 0.05)(D, F)),
            "w_down": _w((lambda *s: _rng.normal(s) * 0.05)(F, D)),
        }
    _B_in = _B_setup()

    return {
        "A_x": _A_in["x"],
        "A_wqkv": _A_in["wqkv"],
        "A_wo": _A_in["wo"],
        "B_x": _B_in["x"],
        "B_w_gate": _B_in["w_gate"],
        "B_w_up": _B_in["w_up"],
        "B_w_down": _B_in["w_down"],
    }

def reference(A_x, A_wqkv, A_wo, B_x, B_w_gate, B_w_up, B_w_down):
    def _A_ref(x, wqkv, wo):
        B, S, D = x.shape
        H = 32; Dh = D // H
        qkv = (lambda x, *d: x.transpose(*d))((x @ wqkv).reshape(B, S, 3, H, Dh), 2, 0, 3, 1, 4)
        q, k, v = qkv[0], qkv[1], qkv[2]
        scale = Dh ** -0.5
        scores = jnp.einsum("bhqd,bhkd->bhqk", q, k) * scale
        p = _softmax(scores, axis=-1)
        o = jnp.einsum("bhqk,bhkd->bhqd", p, v)
        return (lambda x, *d: x.transpose(*d))(o, 0, 2, 1, 3).reshape(B, S, D) @ wo

    def _B_ref(x, w_gate, w_up, w_down):
        g = _silu(x @ w_gate)
        u = x @ w_up
        return (g * u) @ w_down

    x = A_x
    h = x + _A_ref(_layernorm(x, axis=-1), A_wqkv, A_wo)
    h2 = h + _B_ref(_layernorm(h, axis=-1), B_w_gate, B_w_up, B_w_down)
    return h2
```

```python
import jax
import jax.numpy as jnp
from jax import lax
import jax.experimental.pallas as pl
import jax.experimental.pallas.tpu as pltpu

_H = 32
_EPS = 1e-5
_LOG2E = 1.4426950408889634
_R = 512
_CK = 128
_G = 32
F32 = jnp.float32
BF16 = jnp.bfloat16


def _ln(x):
    d = x - jnp.mean(x, axis=-1, keepdims=True)
    return d * lax.rsqrt(jnp.mean(d * d, axis=-1, keepdims=True) + _EPS)


def _mo(i, n):
    return i if isinstance(i, int) else pl.multiple_of(i, n)


def _dot(a, b):
    return jnp.dot(a, b, preferred_element_type=F32)


def _fold(reduce, combine, a, cur):
    r = reduce(a.reshape(a.shape[0] // 8, 8, a.shape[1]), axis=0)
    return r if cur is None else combine(cur, r)


def _strassen_lhs(a11, a12, a21, a22):
    return [t.astype(BF16) for t in (a11 + a22, a21 + a22, a11, a22, a11 + a12, a21 - a11, a12 - a22)]


def _strassen_rhs(b11, b12, b21, b22):
    b11, b12, b21, b22 = (b.astype(F32) for b in (b11, b12, b21, b22))
    return [t.astype(BF16) for t in (b11 + b22, b12 - b22, b21 - b11, b11 + b12, b21 + b22)]


def _rhs_order(sums, b11, b22):
    return [sums[0], b11, sums[1], sums[2], b22, sums[3], sums[4]]


def _strassen_out(m):
    return (m[0] + m[3]) + (m[6] - m[4]), m[2] + m[4], m[1] + m[3], (m[0] - m[1]) + (m[2] + m[5])


def _silu(g):
    hg = 0.5 * g
    return hg + hg * jnp.tanh(hg)


def _run(gen):
    for _ in gen:
        pass


@jax.jit
def pallas_sequential_preLN__softmax_full_mha__swiglu_ffn__prompt_kernel(
    A_x, A_wqkv, A_wo, B_x, B_w_gate, B_w_up, B_w_down
):
    del B_x
    _, S, D = A_x.shape
    F = B_w_gate.shape[1]
    H, R, CK, G = _H, _R, _CK, _G
    Dh = D // H
    NB, NC, HG = S // R, S // CK, 128 // Dh
    HD, HR, HF, NF = D // 2, R // 2, F // 2, F // 256
    PIECE = HR // 8
    qscale = float(Dh ** -0.5 * _LOG2E)

    def body(x_hbm, wqkv_hbm, wo_hbm, wg_hbm, wu_hbm, wd_hbm, out_hbm,
             x_v, w4_v, wg_v, wu_v, wd_v, out_v, h_s, k_s, qt_s, vt_s, ot_s, s_s, p_s, m_s, l_s,
             w3_s, w1_s, w2_s, a1_s, a2_s, a3_s, kall_s, sem_x, sem_w, sem_o):
        def rows_of(i, r=0, n=R):
            return pl.ds(_mo(i * R + r, n), n)

        x_cp = [pltpu.make_async_copy(x_hbm.at[rows_of(i)], x_v.at[rows_of(i)], sem_x.at[i]) for i in range(NB)]
        qkv_cp = [pltpu.make_async_copy(wqkv_hbm.at[:, pl.ds(i * D, D)], w4_v.at[i], sem_w.at[i]) for i in range(3)]
        w_cp = [pltpu.make_async_copy(a, b, sem_w.at[3 + i]) for i, (a, b) in enumerate(
            ((wo_hbm, w4_v.at[3]), (wg_hbm, wg_v), (wu_hbm, wu_v), (wd_hbm, wd_v)))]

        def quadrants_to(dst, rows, r):
            for e, t in enumerate(_strassen_lhs(*[v[:, k * HD:(k + 1) * HD] for v in rows for k in (0, 1)])):
                dst[e, pl.ds(r, PIECE), :] = t

        def ln_block(src, i, dst=a1_s):
            for r in range(0, HR, PIECE):
                quadrants_to(dst, [_ln(src[rows_of(i, k * HR + r, PIECE), :].astype(F32)) for k in (0, 1)], r)
                yield

        def prep_square(i):
            b = [w4_v[i, pl.ds(a * HD, HD), pl.ds(k * HD, HD)] for a in (0, 1) for k in (0, 1)]
            for e, t in enumerate(_rhs_order(_strassen_rhs(*b), b[0], b[3])):
                w3_s[i, e] = t if i == 1 else t.T

        def dot_square_t(i):
            c = _strassen_out([lax.dot_general(w3_s[i, e], a1_s[e], (((1,), (1,)), ((), ())),
                                               preferred_element_type=F32) for e in range(7)])
            return jnp.concatenate([jnp.concatenate([c[0], c[2]], axis=1), jnp.concatenate([c[1], c[3]], axis=1)], axis=0)

        def dot_square(i):
            c = _strassen_out([_dot(a1_s[e], w3_s[i, e]) for e in range(7)])
            return jnp.concatenate([jnp.concatenate(c[0:2], axis=1), jnp.concatenate(c[2:4], axis=1)], axis=0)

        def project(i, before):
            before(1)
            k = pltpu.bitcast(dot_square(1).astype(BF16), jnp.uint32)
            for g in range(D // 128):
                kall_s[g, pl.ds(_mo(i * (R // 2), R // 2), R // 2), :] = k[:, g * 128:(g + 1) * 128]
            before(0)
            qt_s[i] = (dot_square_t(0) * qscale).astype(BF16).reshape(H, Dh, R)
            before(2)
            vt = dot_square_t(2).astype(BF16)
            for c in range(R // CK):
                vt_s[i * (R // CK) + c] = vt[:, c * CK:(c + 1) * CK].reshape(H, Dh, CK)

        def arrive(n):
            qkv_cp[n].wait()
            for c in {1: [qkv_cp[2], x_cp[1]], 0: x_cp[2:], 2: []}[n]:
                c.start()
            prep_square(n)

        x_cp[0].start()
        qkv_cp[1].start()
        x_cp[0].wait()
        qkv_cp[0].start()
        _run(ln_block(x_v, 0))

        def next_operands():
            for e in range(7):
                a1_s[e] = a3_s[e]

        def arrive_first(n):
            arrive(n)
            if n == 2:
                x_cp[1].wait()
                _run(ln_block(x_v, 1, a3_s))

        project(0, arrive_first)
        next_operands()
        for c in x_cp[2:]:
            c.wait()
        for c in w_cp:
            c.start()

        @pl.loop(1, NB)
        def _(i):
            def before(n):
                if n == 2:
                    _run(ln_block(x_v, jnp.minimum(i + 1, NB - 1), a3_s))

            project(i, before)
            next_operands()

        def load_keys(h, c):
            words = pl.ds(c * CK // 2, CK // 2)
            k_s[words, :] = pltpu.roll(kall_s[h // HG, words, :], (128 - h % HG * Dh) % 128, 1)

        def step(j, h, do_qk=True, do_exp=True, do_pv=True):
            m8 = l8 = acc = None
            if do_qk:
                w = qt_s[j, h + 2]
            if do_exp:
                m = jnp.max(m_s[j], axis=0, keepdims=True)
            if do_pv:
                inv = 1.0 / jnp.sum(l_s[j], axis=0, keepdims=True)
            for c in range(NC):
                if do_pv:
                    o = _dot(vt_s[c, h], p_s[j, pl.ds(c * CK, CK), :])
                    acc = o if acc is None else acc + o
                if do_qk:
                    s = _dot(pltpu.bitcast(k_s[pl.ds(c * CK // 2, CK // 2), :], BF16)[:, 0:Dh], w)
                    if j == 0 and c < NC // 2:
                        load_keys(h + 2, c + NC // 2)
                    if j == NB - 1 and NC // 4 <= c < NC // 4 + NC // 2:
                        load_keys(jnp.minimum(h + 3, H - 1), c - NC // 4)
                for r in range(0, CK, G):
                    keys = pl.ds(c * CK + r, G)
                    if do_exp:
                        p = jnp.exp2(s_s[j, keys, :] - m)
                        l8 = _fold(jnp.sum, jnp.add, p, l8)
                        p_s[j, keys, :] = p.astype(BF16)
                    if do_qk:
                        s_s[j, keys, :] = s[r:r + G]
                        m8 = _fold(jnp.max, jnp.maximum, s[r:r + G], m8)
                if c < NC - 1:
                    yield
            if do_qk:
                m_s[j] = m8
            if do_exp:
                l_s[j] = l8
            if do_pv:
                ot_s[j, pl.ds(_mo(h * Dh, Dh), Dh), :] = acc * inv
            yield

        def prep_weights(h, n):
            r = _mo(jnp.minimum(h, HD // 16 - 1) * 16, 16)
            if n < F // 128:
                cols = pl.ds(n * 128, 128)
                b = [ref[pl.ds(k * HD + r, 16), cols] for k in (0, 1) for ref in (wg_v, wu_v)]
                for e, t in enumerate(_strassen_rhs(*b)):
                    w1_s[e, pl.ds(r, 16), cols] = t
            elif n < F // 128 + HD // 128:
                r, c0 = _mo(jnp.minimum(h, HF // 32 - 1) * 32, 32), (n - F // 128) * 128
                b = [wd_v[pl.ds(a * HF + r, 32), pl.ds(k * HD + c0, 128)] for a in (0, 1) for k in (0, 1)]
                for e, t in enumerate(_strassen_rhs(*b)):
                    w2_s[e, pl.ds(r, 32), pl.ds(c0, 128)] = t

        def drain(j):
            yield from step(j, H - 2, do_qk=False)
            o0 = ot_s[j, 0:D - 128, :].T
            yield from step(j, H - 1, do_qk=False, do_exp=False)
            o = jnp.concatenate([o0, ot_s[j, D - 128:D, :].T], axis=1)
            y = _dot(o.astype(BF16), w4_v[3])
            h_s[rows_of(j), :] = x_v[rows_of(j), :].astype(F32) + y
            yield

        k_s[...] = kall_s[0]
        for j in range(NB):
            _run(step(j, -2, do_exp=False, do_pv=False))
        for j in range(NB):
            _run(step(j, -1, do_pv=False))
        for c in w_cp:
            c.wait()
        assert H - 3 >= max(HD // 16, HF // 32)

        @pl.loop(0, H - 2)
        def _(h):
            for j in range(NB):
                for c, _ in enumerate(step(j, h)):
                    if c % 2 == 1:
                        prep_weights(h, (j * NC + c) // 2)

        _run(drain(0))
        _run(ln_block(h_s, 0))

        def out_cp(i, k):
            rows = rows_of(i, k * HR, HR)
            return pltpu.make_async_copy(out_v.at[rows], out_hbm.at[rows], sem_o.at[i, k])

        def ffn(i, more=True):
            side, side2 = (drain(i + 1), ln_block(h_s, i + 1)) if more else (iter(()), iter(()))

            def activate(ms, f, n):
                g1, u1, g2, u2 = _strassen_out([t[n * PIECE:(n + 1) * PIECE] for t in ms])
                y1, y2 = _silu(g1) * u1, _silu(g2) * u2
                for e, t in enumerate(_strassen_lhs(y1[:, :128], y1[:, 128:], y2[:, :128], y2[:, 128:])):
                    a2_s[e, pl.ds(n * PIECE, PIECE), pl.ds(f * 128, 128)] = t

            prev = None
            ws = _rhs_order([w1_s.at[e] for e in range(5)], wg_v.at[0:HD], wu_v.at[HD:D])
            for f in range(NF):
                ms = []
                for e in range(7):
                    w = jnp.concatenate([ws[e][:, pl.ds(k * HF + f * 128, 128)] for k in (0, 1)], axis=1)
                    ms.append(_dot(a1_s[e], w))
                    if f:
                        activate(prev, f - 1, e)
                    if e < 4 + (f >= NF - 3):
                        next(side, None)
                if f:
                    activate(prev, f - 1, 7)
                prev = ms
            _run(side)
            for n in range(8):
                activate(prev, NF - 1, n)
            ws = _rhs_order([w2_s.at[e] for e in range(5)], wd_v.at[0:HF, 0:HD], wd_v.at[HF:F, HD:D])
            ks = HF - 256
            ms = []
            for e in range(7):
                ms.append(_dot(a2_s[e, :, 0:ks], ws[e][0:ks, :]))
                next(side2, None)
            _run(side2)
            for e in (1, 3, 0, 2, 5, 4, 6):
                ms[e] = ms[e] + _dot(a2_s[e, :, ks:], ws[e][ks:, :])
            cs = _strassen_out(ms)
            for k in (1, 0):
                for n in (0, 1):
                    blk = (rows_of(i, k * HR, HR), pl.ds(n * HD, HD))
                    out_v[blk] = (h_s[blk] + cs[2 * k + n]).astype(out_v.dtype)
                if not more:
                    out_cp(i, k).start()
            if more:
                out_cp(i, 0).start()
                out_cp(i, 1).start()

        pl.loop(0, NB - 1)(ffn)
        ffn(NB - 1, more=False)
        for i in range(NB):
            for k in (0, 1):
                out_cp(i, k).wait()

    any_spec = pl.BlockSpec(memory_space=pl.ANY)
    out = pl.pallas_call(
        body,
        in_specs=[any_spec] * 6,
        out_specs=any_spec,
        out_shape=jax.ShapeDtypeStruct((S, D), A_x.dtype),
        scratch_shapes=[
            pltpu.VMEM((S, D), A_x.dtype),
            pltpu.VMEM((4, D, D), BF16),
            pltpu.VMEM((D, F), BF16),
            pltpu.VMEM((D, F), BF16),
            pltpu.VMEM((F, D), BF16),
            pltpu.VMEM((S, D), A_x.dtype),
            pltpu.VMEM((S, D), F32),
            pltpu.VMEM((S // 2, 128), jnp.uint32),
            pltpu.VMEM((NB, H, Dh, R), BF16),
            pltpu.VMEM((NC, H, Dh, CK), BF16),
            pltpu.VMEM((NB, D, R), F32),
            pltpu.VMEM((NB, S, R), F32),
            pltpu.VMEM((NB, S, R), BF16),
            pltpu.VMEM((NB, 8, R), F32),
            pltpu.VMEM((NB, 8, R), F32),
            pltpu.VMEM((3, 7, HD, HD), BF16),
            pltpu.VMEM((5, HD, F), BF16),
            pltpu.VMEM((5, HF, HD), BF16),
            pltpu.VMEM((7, HR, HD), BF16),
            pltpu.VMEM((7, HR, HF), BF16),
            pltpu.VMEM((7, HR, HD), BF16),
            pltpu.VMEM((D // 128, S // 2, 128), jnp.uint32),
            pltpu.SemaphoreType.DMA((NB,)),
            pltpu.SemaphoreType.DMA((7,)),
            pltpu.SemaphoreType.DMA((NB, 2)),
        ],
        compiler_params=pltpu.CompilerParams(vmem_limit_bytes=100 * 1024 * 1024),
    )(A_x.reshape(S, D), A_wqkv.astype(BF16), A_wo.astype(BF16),
      B_w_gate.astype(BF16), B_w_up.astype(BF16), B_w_down.astype(BF16))
    return out.reshape(A_x.shape)
```
